```python
import os as _os
_os.environ.setdefault("JAX_PLATFORMS", "cpu")
import jax
import jax.numpy as jnp

def _softmax(x, axis=-1):
    return jax.nn.softmax(x, axis=axis)
def _gelu(x):
    return jax.nn.gelu(x, approximate=True)
def _silu(x):
    return jax.nn.silu(x)
def _sigmoid(x):
    return jax.nn.sigmoid(x)
def _layernorm(x, axis=-1, eps=1e-5):
    m = jnp.mean(x, axis=axis, keepdims=True)
    v = jnp.var(x, axis=axis, keepdims=True)
    return (x - m) / jnp.sqrt(v + eps)
def _scatter_add(tgt, idx, src, axis=0):
    return tgt.at[idx].add(src)
def _segment_sum(src, seg, n):
    return jax.ops.segment_sum(src, seg, n)
class _Rng:
    def __init__(self, key):
        self._k = key
    def _next(self):
        self._k, sub = jax.random.split(self._k)
        return sub
    def normal(self, shape):
        return jax.random.normal(self._next(), shape, dtype=jnp.bfloat16)
    def randint(self, lo, hi, shape):
        return jax.random.randint(self._next(), shape, lo, hi, dtype=jnp.int32)
    def uniform(self, shape, lo=0.0, hi=1.0):
        return jax.random.uniform(self._next(), shape, jnp.bfloat16, lo, hi)
    def permutation(self, n):
        return jax.random.permutation(self._next(), n)


kernel_name = 'standalone__se_block__vision'

def setup_inputs():
    _rng = _Rng(jax.random.key(int.from_bytes(__import__("os").urandom(4), "little")))
    _w = (lambda a: (lambda t: t.astype(jnp.bfloat16) if jnp.issubdtype(t.dtype, jnp.floating) else t)(jnp.asarray(a)))
    H = W = 384
    C = 192; r = max(C // 16, 4)
    return {
        "x": _w((lambda *s: _rng.normal(s) * 0.8)(1, H, W, C)),
        "w_down": _w((lambda *s: _rng.normal(s) * 0.8)(C, r)),
        "w_up": _w((lambda *s: _rng.normal(s) * 0.8)(r, C)),
    }

def reference(x, w_down, w_up):
    s = x.mean(axis=(1, 2))
    s = _sigmoid(_silu(s @ w_down) @ w_up)
    return x * s[:, None, None, :]
```

```python
import jax
import jax.numpy as jnp
from jax import lax
import jax.experimental.pallas as pl
import jax.experimental.pallas.tpu as pltpu

LANES = 128
SUBLANES = 8


@jax.jit
def pallas_standalone__se_block__vision_kernel(
    x: jax.Array,
    w_down: jax.Array,
    w_up: jax.Array,
):
    n, h, w, c = x.shape
    r = w_down.shape[1]
    assert n == 1 and c % SUBLANES == 0 and w % LANES == 0
    cg = c // SUBLANES
    lt = w // LANES
    slab_rows = c * lt

    read_chunks = (192, 128, 48, 12, 3, 1)
    run_rows, n_pass = 64, 128
    assert sum(read_chunks) == h
    n_blk = h * slab_rows // (run_rows * n_pass)
    assert n_blk * run_rows * n_pass == h * slab_rows and slab_rows % run_rows == 0
    period = slab_rows // run_rows
    wshape = (n_blk, n_pass, run_rows, LANES)

    def kernel(x_hbm, wd_hbm, wu_hbm, o_hbm, buf, wd_v, wu_v, tab, rsem, wsem):
        slabs = buf.reshape(h, slab_rows, LANES)
        reads = []
        h0 = 0
        for i, size in enumerate(read_chunks):
            reads.append(pltpu.make_async_copy(
                x_hbm.at[pl.ds(h0, size)], slabs.at[pl.ds(h0, size)], rsem.at[i]))
            h0 += size
        wd_cp = pltpu.make_async_copy(wd_hbm, wd_v, wsem.at[0])
        wu_cp = pltpu.make_async_copy(wu_hbm, wu_v, wsem.at[1])
        wd_cp.start()
        wu_cp.start()
        for cp in reads:
            cp.start()

        def accumulate(i, acc):
            acc = list(acc)
            for k in range(slab_rows // 16):
                v = slabs[i, pl.ds(16 * k, 16), :].astype(jnp.float32)
                acc[(2 * k) // lt] = acc[(2 * k) // lt] + v[:8]
                acc[(2 * k + 1) // lt] = acc[(2 * k + 1) // lt] + v[8:]
            return tuple(acc)

        acc = tuple(jnp.zeros((SUBLANES, LANES), jnp.float32) for _ in range(cg))
        h0 = 0
        for i, size in enumerate(read_chunks):
            reads[i].wait()
            if i == 3:
                wd_cp.wait()
                wu_cp.wait()
                wdt = wd_v[...]
                wut = wu_v[...].astype(jnp.float32).T.astype(jnp.bfloat16)
            if size <= 3:
                for j in range(h0, h0 + size):
                    acc = accumulate(j, acc)
            else:
                acc = lax.fori_loop(h0, h0 + size, accumulate, acc)
            h0 += size

        def round_bf16(v):
            return v.astype(jnp.bfloat16).astype(jnp.float32)

        total = jnp.concatenate(acc, axis=0)
        mean = jnp.sum(total, axis=1, keepdims=True) * (1.0 / (h * w))
        mean = jnp.broadcast_to(mean, (c, LANES)).astype(jnp.bfloat16)
        hid = round_bf16(jnp.dot(wdt, mean, preferred_element_type=jnp.float32))
        act = (hid * round_bf16(jax.nn.sigmoid(hid))).astype(jnp.bfloat16)
        z = round_bf16(jnp.dot(wut, act, preferred_element_type=jnp.float32))
        s = round_bf16(jax.nn.sigmoid(z))

        for rep in range(2):
            for t in range(cg * lt):
                g = t // lt
                tab[pl.ds(rep * slab_rows + 8 * t, 8), :] = s[8 * g: 8 * g + 8]

        def scale_pass(j, jm):
            for a in range(n_blk):
                off = ((a * n_pass) % period) * run_rows
                base = pl.multiple_of(jm * run_rows + off, run_rows)
                v = buf[a, j].astype(jnp.float32) * tab[pl.ds(base, run_rows), :]
                buf[a, j] = v.astype(jnp.bfloat16)
            pltpu.make_async_copy(buf.at[:, j], o_hbm.at[:, j], wsem.at[0]).start()
            jm = jm + 1
            return jnp.where(jm == period, 0, jm)

        lax.fori_loop(0, n_pass, scale_pass, 0)
        pltpu.make_async_copy(buf, o_hbm, wsem.at[0]).wait()

    xt = jnp.transpose(x, (0, 1, 3, 2)).reshape(h, cg, SUBLANES, lt, LANES)
    xt = jnp.transpose(xt, (0, 1, 3, 2, 4)).reshape(h, slab_rows, LANES)
    hbm = pl.BlockSpec(memory_space=pltpu.HBM)
    out = pl.pallas_call(
        kernel,
        out_shape=jax.ShapeDtypeStruct(wshape, x.dtype),
        in_specs=[hbm, hbm, hbm],
        out_specs=hbm,
        scratch_shapes=[
            pltpu.VMEM(wshape, x.dtype),
            pltpu.VMEM((r, c), w_down.dtype),
            pltpu.VMEM((r, c), w_up.dtype),
            pltpu.VMEM((2 * slab_rows, LANES), jnp.float32),
            pltpu.SemaphoreType.DMA((len(read_chunks),)),
            pltpu.SemaphoreType.DMA((2,)),
        ],
        compiler_params=pltpu.CompilerParams(vmem_limit_bytes=80 * 1024 * 1024),
        name="se_block",
    )(xt, w_down.T, w_up)
    out = jnp.transpose(out.reshape(h, cg, lt, SUBLANES, LANES), (0, 1, 3, 2, 4))
    return jnp.transpose(out.reshape(n, h, c, w), (0, 1, 3, 2))
```

```python
import jax
import jax.numpy as jnp
from jax import lax
import jax.experimental.pallas as pl
import jax.experimental.pallas.tpu as pltpu

LANES = 128
TILE = 8
PACK = 16

RUN_ROWS = 64
BLOCK_RUNS = 64
STREAMS = 6

FULL_CHUNKS = (128, 48, 16)
TAIL_CHUNKS = (12, 3, 1)
LATE_CHUNKS = (13, 3)
LATE_GROUPS = 2


def _tree_sum(values):
    values = list(values)
    while len(values) > 1:
        values = [sum(values[i + 1:i + 2], values[i]) for i in range(0, len(values), 2)]
    return values[0]


def _ranges(start, sizes):
    out = []
    for size in sizes:
        out.append((start, size))
        start += size
    return out


@jax.jit
def pallas_standalone__se_block__vision_kernel(
    x: jax.Array,
    w_down: jax.Array,
    w_up: jax.Array,
):
    n, h, w, c = x.shape
    hidden = w_down.shape[1]
    f32 = jnp.float32

    groups = c // TILE
    lane_tiles = w // LANES
    slab_rows = c * lane_tiles
    run_tiles = RUN_ROWS // TILE
    phases = slab_rows // RUN_ROWS
    blocks = h * phases // BLOCK_RUNS
    late_rows = LATE_GROUPS * lane_tiles * TILE
    late_row0 = slab_rows - late_rows
    late_channels = LATE_GROUPS * TILE
    tail = sum(TAIL_CHUNKS)
    table_len = phases + STREAMS - 1

    assert n == 1 and groups * TILE == c and lane_tiles * LANES == w
    assert phases * RUN_ROWS == slab_rows and blocks * BLOCK_RUNS == h * phases
    assert blocks % STREAMS == 0 and blocks % phases == 0
    assert BLOCK_RUNS % phases == 1
    assert late_rows % PACK == 0 and sum(LATE_CHUNKS) == tail
    assert h > tail + sum(FULL_CHUNKS)

    slab_shape = (h, slab_rows, LANES)
    block_shape = (blocks, BLOCK_RUNS, RUN_ROWS, LANES)
    phase_shape = (blocks // phases, phases, BLOCK_RUNS, RUN_ROWS, LANES)

    def kernel(x_hbm, wd_hbm, wu_hbm, o_hbm,
               buf, wd_ref, wu_ref, wu_f32, wu_tiles, wd_late, hid_ref, table, write_sem):

        def broadcast_weights():
            wu_f32[...] = wu_ref[...].astype(f32)

            @pl.loop(0, hidden)
            def _(r):
                col = jnp.broadcast_to(wu_f32[pl.ds(r, 1), :], (LANES, c)).T
                for t in range(slab_rows // TILE):
                    c0 = t // lane_tiles * TILE
                    rows = pl.ds(t % run_tiles * TILE, TILE)
                    wu_tiles[r, t // run_tiles, rows, :] = col[c0:c0 + TILE]

            wd = wd_ref[...].astype(f32) * (1.0 / (h * w))
            for i in range(late_channels):
                ch = c - late_channels + i
                wd_late[i] = jnp.broadcast_to(wd[:, ch:ch + 1], (hidden, LANES))

        def add_slabs(acc, start, size, rows):
            def add_slab(i, acc):
                acc = list(acc)
                for row in range(0, rows, PACK):
                    v = slabs[i, pl.ds(row, PACK), :].astype(f32)
                    for k in range(0, PACK, TILE):
                        g = (row + k) // TILE // lane_tiles
                        acc[g] = acc[g] + v[k:k + TILE]
                return tuple(acc)

            if size > 3:
                return lax.fori_loop(start, start + size, add_slab, acc)
            for i in range(start, start + size):
                acc = add_slab(i, acc)
            return acc

        def scale_run(ref, idx, scale):
            ref[idx] = (ref[idx].astype(f32) * scale).astype(ref.dtype)

        def write(src, dst, idx):
            pltpu.make_async_copy(src.at[idx], dst.at[idx], write_sem).start()

        slabs = buf.reshape(slab_shape)
        buf_by_phase = buf.reshape(phase_shape)
        out_by_phase = o_hbm.reshape(phase_shape)

        full = _ranges(0, (h - tail - sum(FULL_CHUNKS),) + FULL_CHUNKS)
        early = _ranges(h - tail, TAIL_CHUNKS)
        late = _ranges(h - tail, LATE_CHUNKS)
        num_reads = len(full) + len(early) + len(late) + 2

        def squeeze_excite(read_sems):
            sems = (read_sems.at[i] for i in range(num_reads))

            def read(ranges, row0, rows):
                idxs = [(pl.ds(start, size), pl.ds(row0, rows)) for start, size in ranges]
                return [pltpu.make_async_copy(x_hbm.at[i], slabs.at[i], next(sems)) for i in idxs]

            full_reads = read(full, 0, slab_rows)
            early_reads = read(early, 0, late_row0)
            late_reads = read(late, late_row0, late_rows)
            weight_reads = [
                pltpu.make_async_copy(wd_hbm, wd_ref, next(sems)),
                pltpu.make_async_copy(wu_hbm, wu_ref, next(sems)),
            ]
            for copy in full_reads[:1] + weight_reads + full_reads[1:] + early_reads + late_reads:
                copy.start()

            acc = tuple(jnp.zeros((TILE, LANES), f32) for _ in range(groups))
            for i, (copy, (start, size)) in enumerate(zip(full_reads, full)):
                copy.wait()
                if i == 0:
                    for weight_read in weight_reads:
                        weight_read.wait()
                    broadcast_weights()
                acc = add_slabs(acc, start, size, slab_rows)
            for copy, (start, size) in zip(early_reads, early):
                copy.wait()
                acc = add_slabs(acc, start, size, late_row0)
            mean = jnp.sum(jnp.concatenate(acc, axis=0), axis=1, keepdims=True) * (1.0 / (h * w))
            mean = jnp.broadcast_to(mean, (c, LANES)).astype(wd_ref.dtype)
            hid = jnp.dot(wd_ref[...], mean, preferred_element_type=f32)

            parts = [[] for _ in range(LATE_GROUPS)]
            for i, (copy, (start, size)) in enumerate(zip(late_reads, late)):
                if i == len(late) - 1:
                    hid_ref[...] = hid
                copy.wait()
                tiles = [None] * (2 * late_rows // TILE)
                for j in range(start, start + size):
                    v = slabs[j, pl.ds(late_row0, late_rows), :].astype(f32)
                    for t in range(late_rows // TILE):
                        k, tile = 2 * t + j % 2, v[t * TILE:(t + 1) * TILE]
                        tiles[k] = tile if tiles[k] is None else tiles[k] + tile
                for g in range(LATE_GROUPS):
                    mine = tiles[2 * lane_tiles * g:2 * lane_tiles * (g + 1)]
                    parts[g] = [_tree_sum([t for t in mine if t is not None] + parts[g])]
            terms = [hid_ref[...]]
            for g in range(LATE_GROUPS):
                total = jnp.sum(parts[g][0], axis=1, keepdims=True)
                total = jnp.broadcast_to(total, (TILE, LANES))
                terms += [total[i:i + 1] * wd_late[g * TILE + i] for i in range(TILE)]
            hid = _tree_sum(terms)

            act = hid * jax.nn.sigmoid(hid)
            act = [jnp.broadcast_to(act[r:r + 1], (TILE, LANES)) for r in range(hidden)]

            def gate(phase, t):
                rows = pl.ds(t * TILE, TILE)
                return jax.nn.sigmoid(
                    _tree_sum(act[r] * wu_tiles[r, phase, rows, :] for r in range(hidden)))

            def write_phase(phase, scale, start, size):
                for q in range(start, start + size):
                    scale_run(buf_by_phase, (q, phase, 0), scale)
                write(buf_by_phase, out_by_phase, (pl.ds(start, size), phase, 0))

            gates = {t: gate(0, t) for t in range(0, run_tiles, lane_tiles)}
            scale = jnp.concatenate([gates[t - t % lane_tiles] for t in range(run_tiles)], axis=0)
            write_phase(0, scale, 0, 1)
            write_phase(0, scale, 1, blocks // phases - 1)

            def next_phase(phase, previous):
                table[phase - 1] = previous
                scale = jnp.concatenate([gate(phase, t) for t in range(run_tiles)], axis=0)
                write_phase(phase, scale, 0, blocks // phases)
                return scale

            table[phases - 1] = lax.fori_loop(1, phases, next_phase, scale)
            for phase in range(phases, table_len):
                table[phase] = table[phase - phases]

            def next_runs(_, carry):
                block, run, phase = carry
                for i in range(STREAMS):
                    scale_run(buf, (block + i, run), table[phase + i])
                write(buf, o_hbm, (pl.ds(block, STREAMS), run))
                wrap = run == BLOCK_RUNS - 1
                phase = phase + jnp.where(wrap, (STREAMS + 1) % phases, 1)
                return (
                    jnp.where(wrap, block + STREAMS, block),
                    jnp.where(wrap, 1, run + 1),
                    jnp.where(phase >= phases, phase - phases, phase),
                )

            lax.fori_loop(0, blocks // STREAMS * (BLOCK_RUNS - 1), next_runs, (0, 1, 1))

        pl.run_scoped(squeeze_excite, pltpu.SemaphoreType.DMA((num_reads,)))
        pltpu.make_async_copy(buf, o_hbm, write_sem).wait()

    xt = jnp.transpose(x, (0, 1, 3, 2)).reshape(h, groups, TILE, lane_tiles, LANES)
    xt = jnp.transpose(xt, (0, 1, 3, 2, 4)).reshape(slab_shape)
    hbm = pl.BlockSpec(memory_space=pltpu.HBM)
    out = pl.pallas_call(
        kernel,
        out_shape=jax.ShapeDtypeStruct(block_shape, x.dtype),
        in_specs=[hbm, hbm, hbm],
        out_specs=hbm,
        scratch_shapes=[
            pltpu.VMEM(block_shape, x.dtype),
            pltpu.VMEM((hidden, c), w_down.dtype),
            pltpu.VMEM((hidden, c), w_up.dtype),
            pltpu.VMEM((hidden, c), f32),
            pltpu.VMEM((hidden, phases, RUN_ROWS, LANES), f32),
            pltpu.VMEM((late_channels, hidden, LANES), f32),
            pltpu.VMEM((hidden, LANES), f32),
            pltpu.VMEM((table_len, RUN_ROWS, LANES), f32),
            pltpu.SemaphoreType.DMA,
        ],
        compiler_params=pltpu.CompilerParams(vmem_limit_bytes=80 * 1024 * 1024),
        name="se_block",
    )(xt, w_down.T, w_up)
    out = out.reshape(h, groups, lane_tiles, TILE, LANES)
    out = jnp.transpose(out, (0, 1, 3, 2, 4)).reshape(n, h, c, w)
    return jnp.transpose(out, (0, 1, 3, 2))
```
